```python
import os as _os
_os.environ.setdefault("JAX_PLATFORMS", "cpu")
import jax
import jax.numpy as jnp

def _softmax(x, axis=-1):
    return jax.nn.softmax(x, axis=axis)
def _gelu(x):
    return jax.nn.gelu(x, approximate=True)
def _silu(x):
    return jax.nn.silu(x)
def _sigmoid(x):
    return jax.nn.sigmoid(x)
def _layernorm(x, axis=-1, eps=1e-5):
    m = jnp.mean(x, axis=axis, keepdims=True)
    v = jnp.var(x, axis=axis, keepdims=True)
    return (x - m) / jnp.sqrt(v + eps)
def _scatter_add(tgt, idx, src, axis=0):
    return tgt.at[idx].add(src)
def _segment_sum(src, seg, n):
    return jax.ops.segment_sum(src, seg, n)
class _Rng:
    def __init__(self, key):
        self._k = key
    def _next(self):
        self._k, sub = jax.random.split(self._k)
        return sub
    def normal(self, shape):
        return jax.random.normal(self._next(), shape, dtype=jnp.bfloat16)
    def randint(self, lo, hi, shape):
        return jax.random.randint(self._next(), shape, lo, hi, dtype=jnp.int32)
    def uniform(self, shape, lo=0.0, hi=1.0):
        return jax.random.uniform(self._next(), shape, jnp.bfloat16, lo, hi)
    def permutation(self, n):
        return jax.random.permutation(self._next(), n)


kernel_name = 'gated_mix__linear_attn_block__mixer_token_mlp__prompt'

def setup_inputs():
    _rng = _Rng(jax.random.key(int.from_bytes(__import__("os").urandom(4), "little")))
    _w = (lambda a: (lambda t: t.astype(jnp.bfloat16) if jnp.issubdtype(t.dtype, jnp.floating) else t)(jnp.asarray(a)))
    def _A_setup():
        B, S, D = 1, 2048, 512
        return {
            "x": _w((lambda *s: _rng.normal(s) * 0.05)(B, S, D)),
            "wqkv": _w((lambda *s: _rng.normal(s) * 0.8)(D, 3 * D)),
            "wo": _w((lambda *s: _rng.normal(s) * 0.05)(D, D)),
        }
    _A_in = _A_setup()

    def _B_setup():
        B, S, D, F = 1, 2048, 512, 1792
        return {
            "x": _w((lambda *s: _rng.normal(s) * 0.05)(B, S, D)),
            "w1": _w((lambda *s: _rng.normal(s) * 0.1)(S, F) * (S ** -0.5)),
            "b1": _w((lambda *s: _rng.normal(s) * 0.1)(F) * 0.02),
            "w2": _w((lambda *s: _rng.normal(s) * 0.1)(F, S) * (F ** -0.5)),
            "b2": _w((lambda *s: _rng.normal(s) * 0.1)(S) * 0.02),
        }
    _B_in = _B_setup()

    return {
        "A_x": _A_in["x"],
        "A_wqkv": _A_in["wqkv"],
        "A_wo": _A_in["wo"],
        "B_x": _B_in["x"],
        "B_w1": _B_in["w1"],
        "B_b1": _B_in["b1"],
        "B_w2": _B_in["w2"],
        "B_b2": _B_in["b2"],
        "gate_w": _w((lambda *s: _rng.normal(s) * 0.05)(512) * 16.0),
    }

def reference(A_x, A_wqkv, A_wo, B_x, B_w1, B_b1, B_w2, B_b2, gate_w):
    def _A_ref(x, wqkv, wo):
        B, S, D = x.shape
        H = 32; Dh = D // H
        qkv = (lambda x, *d: x.transpose(*d))((x @ wqkv).reshape(B, S, 3, H, Dh), 2, 0, 3, 1, 4)
        q, k, v = qkv[0], qkv[1], qkv[2]
        phi = lambda t: jnp.where(t > 0, t + 1, jnp.exp(t)) + 1e-6
        pq, pk = phi(q), phi(k)
        kv = jnp.einsum("bhsd,bhse->bhde", pk, v)
        z = jnp.einsum("bhsd->bhd", pk)
        num = jnp.einsum("bhqd,bhde->bhqe", pq, kv)
        den = jnp.einsum("bhqd,bhd->bhq", pq, z)[..., None] + 1e-6
        o = num / den
        return (lambda x, *d: x.transpose(*d))(o, 0, 2, 1, 3).reshape(B, S, D) @ wo

    def _B_ref(x, w1, b1, w2, b2):
        B, S, D = x.shape
        h = _layernorm(x, axis=-1)
        u = jnp.einsum("bsd,sf->bdf", h, w1) + b1
        u = _gelu(u)
        y = jnp.einsum("bdf,fs->bds", u, w2) + b2
        return (lambda x, *d: x.transpose(*d))(y, 0, 2, 1)

    x = A_x
    g = _sigmoid((x * gate_w).sum(-1, keepdims=True))
    a = _A_ref(x, A_wqkv, A_wo)
    b = _B_ref(x, B_w1, B_b1, B_w2, B_b2)
    return g * a + (1 - g) * b
```

```python
import functools

import jax
import jax.numpy as jnp
import jax.experimental.pallas as pl
import jax.experimental.pallas.tpu as pltpu

_LANES = 128


def _kernel(x_ref, wqkv_ref, wo_ref, w1_ref, b1_ref, w2_ref, b2_ref, gw_ref,
            out_ref,
            pq_s, g_s, kv_s, z_s, u_s, gu_s, kvb_s,
            *, nt, ts, d, dh):
    f32 = jnp.float32
    bf16 = jnp.bfloat16
    ng = d // _LANES
    i = pl.program_id(0)

    @pl.when(i < nt)
    def _phase1():
        @pl.when(i == 0)
        def _init():
            kv_s[...] = jnp.zeros_like(kv_s)
            z_s[...] = jnp.zeros_like(z_s)
            u_s[...] = jnp.zeros_like(u_s)

        row0 = pl.multiple_of(i * ts, ts)
        xb = x_ref[...]
        xf = xb.astype(f32)

        gl = jnp.sum(xf * gw_ref[...].astype(f32), axis=-1, keepdims=True)
        g_s[pl.ds(row0, ts), :] = jax.nn.sigmoid(gl)

        m = jnp.mean(xf, axis=-1, keepdims=True)
        xc = xf - m
        var = jnp.mean(xc * xc, axis=-1, keepdims=True)
        h = (xc / jnp.sqrt(var + 1e-5)).astype(bf16)

        u_s[...] += jax.lax.dot_general(
            h, w1_ref[...], (((0,), (0,)), ((), ())),
            preferred_element_type=f32)

        qkv = jnp.dot(xb, wqkv_ref[...], preferred_element_type=f32)
        q = qkv[:, 0 * d:1 * d]
        k = qkv[:, 1 * d:2 * d]
        v = qkv[:, 2 * d:3 * d]
        phi = lambda t: jnp.where(t > 0, t + 1.0, jnp.exp(t)) + 1e-6
        pq_s[pl.ds(row0, ts), :] = phi(q).astype(bf16)
        pk = phi(k)
        z_s[...] += jnp.sum(pk, axis=0, keepdims=True)
        pkb = pk.astype(bf16)
        vb = v.astype(bf16)
        for gidx in range(ng):
            sl = slice(gidx * _LANES, (gidx + 1) * _LANES)
            kv_s[gidx] += jax.lax.dot_general(
                pkb[:, sl], vb[:, sl], (((0,), (0,)), ((), ())),
                preferred_element_type=f32)

    @pl.when(i == nt)
    def _finalize():
        gu_s[...] = jax.nn.gelu(u_s[...] + b1_ref[...].astype(f32),
                                approximate=True).astype(bf16)
        r = jax.lax.broadcasted_iota(jnp.int32, (_LANES, _LANES), 0) // dh
        c = jax.lax.broadcasted_iota(jnp.int32, (_LANES, _LANES), 1) // dh
        same = r == c
        for gidx in range(ng):
            kvb_s[gidx] = jnp.where(same, kv_s[gidx], 0.0).astype(bf16)

    @pl.when(i >= nt)
    def _phase2():
        j = i - nt
        row0 = pl.multiple_of(j * ts, ts)
        r = jax.lax.broadcasted_iota(jnp.int32, (_LANES, _LANES), 0) // dh
        c = jax.lax.broadcasted_iota(jnp.int32, (_LANES, _LANES), 1) // dh
        ones_blk = jnp.where(r == c, 1.0, 0.0).astype(bf16)

        pq = pq_s[pl.ds(row0, ts), :]
        pqz = (pq.astype(f32) * z_s[...]).astype(bf16)
        o_parts = []
        for gidx in range(ng):
            sl = slice(gidx * _LANES, (gidx + 1) * _LANES)
            num = jnp.dot(pq[:, sl], kvb_s[gidx], preferred_element_type=f32)
            den = jnp.dot(pqz[:, sl], ones_blk, preferred_element_type=f32)
            o_parts.append((num / (den + 1e-6)).astype(bf16))
        o = jnp.concatenate(o_parts, axis=-1)
        a = jnp.dot(o, wo_ref[...], preferred_element_type=f32)

        yt = jnp.dot(gu_s[...], w2_ref[...], preferred_element_type=f32)
        yt = yt + b2_ref[...].astype(f32)
        b = yt.T
        g = g_s[pl.ds(row0, ts), :]
        out_ref[...] = (g * a + (1.0 - g) * b).astype(out_ref.dtype)


@jax.jit
def pallas_gated_mix__linear_attn_block__mixer_token_mlp__prompt_kernel(
    A_x: jax.Array,
    A_wqkv: jax.Array,
    A_wo: jax.Array,
    B_x: jax.Array,
    B_w1: jax.Array,
    B_b1: jax.Array,
    B_w2: jax.Array,
    B_b2: jax.Array,
    gate_w: jax.Array,
):
    del B_x
    bsz, s, d = A_x.shape
    assert bsz == 1
    f = B_w1.shape[1]
    n_heads = 32
    dh = d // n_heads
    ts = 256
    nt = s // ts
    ng = d // _LANES

    x = A_x.reshape(s, d)
    b1 = B_b1.reshape(1, f)
    b2 = B_b2.reshape(1, s)
    gw = gate_w.reshape(1, d)

    kern = functools.partial(_kernel, nt=nt, ts=ts, d=d, dh=dh)
    p1 = lambda i: jnp.minimum(i, nt - 1)
    p2 = lambda i: jnp.maximum(i - nt, 0)

    out = pl.pallas_call(
        kern,
        grid=(2 * nt,),
        in_specs=[
            pl.BlockSpec((ts, d), lambda i: (p1(i), 0)),
            pl.BlockSpec((d, 3 * d), lambda i: (0, 0)),
            pl.BlockSpec((d, d), lambda i: (0, 0)),
            pl.BlockSpec((ts, f), lambda i: (p1(i), 0)),
            pl.BlockSpec((1, f), lambda i: (0, 0)),
            pl.BlockSpec((f, ts), lambda i: (0, p2(i))),
            pl.BlockSpec((1, ts), lambda i: (0, p2(i))),
            pl.BlockSpec((1, d), lambda i: (0, 0)),
        ],
        out_specs=pl.BlockSpec((ts, d), lambda i: (p2(i), 0)),
        out_shape=jax.ShapeDtypeStruct((s, d), A_x.dtype),
        scratch_shapes=[
            pltpu.VMEM((s, d), jnp.bfloat16),
            pltpu.VMEM((s, 1), jnp.float32),
            pltpu.VMEM((ng, _LANES, _LANES), jnp.float32),
            pltpu.VMEM((1, d), jnp.float32),
            pltpu.VMEM((d, f), jnp.float32),
            pltpu.VMEM((d, f), jnp.bfloat16),
            pltpu.VMEM((ng, _LANES, _LANES), jnp.bfloat16),
        ],
        compiler_params=pltpu.CompilerParams(
            dimension_semantics=("arbitrary",),
            vmem_limit_bytes=100 * 1024 * 1024,
        ),
    )(x, A_wqkv, A_wo, B_w1, b1, B_w2, b2, gw)
    return out.reshape(1, s, d)
```

```python
import functools

import jax
import jax.numpy as jnp
import jax.experimental.pallas as pl
import jax.experimental.pallas.tpu as pltpu

_LANES = 128


def _kernel(x_hbm, wqkv_hbm, wo_hbm, w1_hbm, w2_hbm, b1_ref, b2_ref, gw_ref,
            out_hbm,
            x_buf, wqkv_buf, wo_buf, w1_buf, w2_buf, ht_s, pq_s, g_s, kv_s, z_s,
            gu_s, m_s, out_buf,
            sem_x, sem_wqkv, sem_wo, sem_w1, sem_w2, sem_out,
            *, s, ts, cf, d, f, dh):
    f32 = jnp.float32
    bf16 = jnp.bfloat16
    nt = s // ts
    nf = f // cf
    ng = d // _LANES

    def x_cp(t):
        return pltpu.make_async_copy(
            x_hbm.at[pl.ds(t * ts, ts), :], x_buf.at[t], sem_x.at[t])

    def w1_cp(c):
        return pltpu.make_async_copy(
            w1_hbm.at[:, pl.ds(c * cf, cf)], w1_buf.at[c], sem_w1.at[c])

    def w2_cp(t):
        return pltpu.make_async_copy(
            w2_hbm.at[:, pl.ds(t * ts, ts)], w2_buf.at[t], sem_w2.at[t])

    def out_cp(t):
        return pltpu.make_async_copy(
            out_buf.at[t % 2], out_hbm.at[pl.ds(t * ts, ts), :], sem_out.at[t % 2])

    def wqkv_cp(j):
        return pltpu.make_async_copy(
            wqkv_hbm.at[:, pl.ds(j * d, d)], wqkv_buf.at[:, pl.ds(j * d, d)],
            sem_wqkv.at[j])

    wo_cp = pltpu.make_async_copy(wo_hbm, wo_buf, sem_wo.at[0])

    x_cp(0).start()
    wqkv_cp(1).start()
    wqkv_cp(2).start()
    wqkv_cp(0).start()
    x_cp(1).start()

    kv_s[...] = jnp.zeros_like(kv_s)
    z_s[...] = jnp.zeros_like(z_s)

    def norm_gate(t):
        row0 = pl.multiple_of(t * ts, ts)
        xf = x_buf[t].astype(f32)
        gl = jnp.sum(xf * gw_ref[...].astype(f32).reshape(1, d), axis=-1, keepdims=True)
        g_s[pl.ds(row0, ts), :] = jax.nn.sigmoid(gl)
        m = jnp.mean(xf, axis=-1, keepdims=True)
        xc = xf - m
        var = jnp.mean(xc * xc, axis=-1, keepdims=True)
        h = xc / jnp.sqrt(var + 1e-5)
        ht_s[:, pl.ds(row0, ts)] = h.T.astype(bf16)

    def attn_stats(t, first=False):
        row0 = pl.multiple_of(t * ts, ts)
        phi = lambda a: jnp.where(a > 0, a + 1.0, jnp.exp(a)) + 1e-6
        if first:
            def proj(j):
                wqkv_cp(j).wait()
                return jnp.dot(x_buf[t], wqkv_buf[:, pl.ds(j * d, d)],
                               preferred_element_type=f32)
            k, v, q = proj(1), proj(2), proj(0)
        else:
            qkv = jnp.dot(x_buf[t], wqkv_buf[...], preferred_element_type=f32)
            q = qkv[:, 0 * d:1 * d]
            k = qkv[:, 1 * d:2 * d]
            v = qkv[:, 2 * d:3 * d]
        pq_s[pl.ds(row0, ts), :] = phi(q).astype(bf16)
        pk = phi(k)
        z_s[...] += jnp.sum(pk, axis=0, keepdims=True)
        pkb = pk.astype(bf16)
        vb = v.astype(bf16)
        for gidx in range(ng):
            sl = slice(gidx * _LANES, (gidx + 1) * _LANES)
            kv_s[gidx] += jax.lax.dot_general(
                pkb[:, sl], vb[:, sl], (((0,), (0,)), ((), ())),
                preferred_element_type=f32)

    x_cp(0).wait()
    norm_gate(0)
    x_cp(2).start()
    w1_cp(0).start()
    attn_stats(0, first=True)
    x_cp(1).wait()
    norm_gate(1)

    def phase_a(t, carry):
        @pl.when(t + 2 < nt)
        def _():
            x_cp(t + 2).start()

        @pl.when(t < nf)
        def _():
            w1_cp(t).start()

        @pl.when(t + 1 < nt)
        def _():
            x_cp(t + 1).wait()
            attn_stats(t)
            norm_gate(t + 1)

        @pl.when(t + 1 == nt)
        def _():
            attn_stats(t)
        return carry

    jax.lax.fori_loop(1, nt, phase_a, 0)

    for c in range(nt, nf):
        w1_cp(c).start()
    wo_cp.start()

    def phase_b(c, carry):
        @pl.when(c < nt)
        def _():
            w2_cp(c).start()

        w1_cp(c).wait()
        col0 = pl.multiple_of(c * cf, cf)
        u = jnp.dot(ht_s[...], w1_buf[c], preferred_element_type=f32)
        u = u + b1_ref[pl.ds(col0, cf)].astype(f32).reshape(1, cf)
        gu_s[:, pl.ds(col0, cf)] = jax.nn.gelu(u, approximate=True).astype(bf16)
        return carry

    jax.lax.fori_loop(0, nf, phase_b, 0)

    for t in range(nf, nt):
        w2_cp(t).start()

    wo_cp.wait()
    r = jax.lax.broadcasted_iota(jnp.int32, (_LANES, _LANES), 0) // dh
    cidx = jax.lax.broadcasted_iota(jnp.int32, (_LANES, _LANES), 1) // dh
    same = r == cidx
    for gidx in range(ng):
        kvb = jnp.where(same, kv_s[gidx], 0.0).astype(bf16)
        m_s[pl.ds(gidx * _LANES, _LANES), :] = jnp.dot(
            kvb, wo_buf[pl.ds(gidx * _LANES, _LANES), :],
            preferred_element_type=f32).astype(bf16)
    ones_blk = jnp.where(same, 1.0, 0.0).astype(bf16)

    def phase_c(t, carry):
        w2_cp(t).wait()

        @pl.when(t >= 2)
        def _():
            out_cp(t - 2).wait()

        row0 = pl.multiple_of(t * ts, ts)
        w2t = w2_buf.at[t]
        parts = []
        yts = []
        for gidx in range(ng):
            sl = slice(gidx * _LANES, (gidx + 1) * _LANES)
            yts.append(jnp.dot(gu_s[sl, :], w2t[...], preferred_element_type=f32))
            pq = pq_s[pl.ds(row0, ts), sl].astype(f32)
            pqz = (pq * z_s[:, sl]).astype(bf16)
            den = jnp.dot(pqz, ones_blk, preferred_element_type=f32)
            parts.append((pq / (den + 1e-6)).astype(bf16))
        yt = jnp.concatenate(yts, axis=0) + b2_ref[pl.ds(row0, ts)].astype(f32).reshape(1, ts)
        b = yt.T
        pqn = jnp.concatenate(parts, axis=-1)
        a = jnp.dot(pqn, m_s[...], preferred_element_type=f32)
        g = g_s[pl.ds(row0, ts), :]
        out_buf[t % 2] = (g * a + (1.0 - g) * b).astype(out_buf.dtype)
        out_cp(t).start()
        return carry

    jax.lax.fori_loop(0, nt, phase_c, 0)
    out_cp(nt - 2).wait()
    out_cp(nt - 1).wait()


@jax.jit
def pallas_gated_mix__linear_attn_block__mixer_token_mlp__prompt_kernel(
    A_x: jax.Array,
    A_wqkv: jax.Array,
    A_wo: jax.Array,
    B_x: jax.Array,
    B_w1: jax.Array,
    B_b1: jax.Array,
    B_w2: jax.Array,
    B_b2: jax.Array,
    gate_w: jax.Array,
):
    del B_x
    bsz, s, d = A_x.shape
    assert bsz == 1
    f = B_w1.shape[1]
    n_heads = 32
    dh = d // n_heads
    ts = 256
    cf = 256
    nt = s // ts
    nf = f // cf
    ng = d // _LANES
    bf16 = jnp.bfloat16

    x = A_x.reshape(s, d)
    b1, b2, gw = B_b1, B_b2, gate_w

    kern = functools.partial(_kernel, s=s, ts=ts, cf=cf, d=d, f=f, dh=dh)
    hbm = pl.BlockSpec(memory_space=pl.ANY)
    out = pl.pallas_call(
        kern,
        in_specs=[hbm, hbm, hbm, hbm, hbm,
                  pl.BlockSpec((f,), lambda: (0,)),
                  pl.BlockSpec((s,), lambda: (0,)),
                  pl.BlockSpec((d,), lambda: (0,))],
        out_specs=hbm,
        out_shape=jax.ShapeDtypeStruct((s, d), A_x.dtype),
        scratch_shapes=[
            pltpu.VMEM((nt, ts, d), bf16),
            pltpu.VMEM((d, 3 * d), bf16),
            pltpu.VMEM((d, d), bf16),
            pltpu.VMEM((nf, s, cf), bf16),
            pltpu.VMEM((nt, f, ts), bf16),
            pltpu.VMEM((d, s), bf16),
            pltpu.VMEM((s, d), bf16),
            pltpu.VMEM((s, 1), jnp.float32),
            pltpu.VMEM((ng, _LANES, _LANES), jnp.float32),
            pltpu.VMEM((1, d), jnp.float32),
            pltpu.VMEM((d, f), bf16),
            pltpu.VMEM((d, d), bf16),
            pltpu.VMEM((2, ts, d), A_x.dtype),
            pltpu.SemaphoreType.DMA((nt,)),
            pltpu.SemaphoreType.DMA((3,)),
            pltpu.SemaphoreType.DMA((1,)),
            pltpu.SemaphoreType.DMA((nf,)),
            pltpu.SemaphoreType.DMA((nt,)),
            pltpu.SemaphoreType.DMA((2,)),
        ],
        compiler_params=pltpu.CompilerParams(
            vmem_limit_bytes=100 * 1024 * 1024,
        ),
    )(x, A_wqkv, A_wo, B_w1, B_w2, b1, b2, gw)
    return out.reshape(1, s, d)
```

```python
import functools

import jax
import jax.numpy as jnp
import jax.experimental.pallas as pl
import jax.experimental.pallas.tpu as pltpu

_LANES = 128


def _kernel(x_hbm, wqkv_hbm, wo_hbm, w1_hbm, w2_hbm, b1_ref, b2_ref, gw_ref,
            out_hbm,
            x_buf, wqkv_buf, wo_buf, w1_buf, w2_buf, ht_s, pq_s, g_s, kv_s, z_s,
            gu_s, m_s, out_buf,
            sem_x, sem_wqkv, sem_wo, sem_w1, sem_w2, sem_out,
            *, s, ts, cf, d, f, dh):
    f32 = jnp.float32
    bf16 = jnp.bfloat16
    nt = s // ts
    nf = f // cf
    ng = d // _LANES

    def x_cp(t):
        return pltpu.make_async_copy(
            x_hbm.at[pl.ds(t * ts, ts), :], x_buf.at[t], sem_x.at[t])

    def w1_cp(c):
        return pltpu.make_async_copy(
            w1_hbm.at[:, pl.ds(c * cf, cf)], w1_buf.at[c], sem_w1.at[c])

    def w2_cp(t):
        return pltpu.make_async_copy(
            w2_hbm.at[:, pl.ds(t * ts, ts)], w2_buf.at[t], sem_w2.at[t])

    def out_cp(t):
        return pltpu.make_async_copy(
            out_buf.at[t % 2], out_hbm.at[pl.ds(t * ts, ts), :], sem_out.at[t % 2])

    def wqkv_cp(j):
        return pltpu.make_async_copy(
            wqkv_hbm.at[:, pl.ds(j * d, d)], wqkv_buf.at[:, pl.ds(j * d, d)],
            sem_wqkv.at[j])

    wo_cp = pltpu.make_async_copy(wo_hbm, wo_buf, sem_wo.at[0])

    x_cp(0).start()
    wqkv_cp(1).start()

    r = jax.lax.broadcasted_iota(jnp.int32, (_LANES, _LANES), 0) // dh
    cidx = jax.lax.broadcasted_iota(jnp.int32, (_LANES, _LANES), 1) // dh
    same = r == cidx
    kv_s[...] = jnp.zeros_like(kv_s)
    z_s[...] = jnp.zeros_like(z_s)

    def norm_gate(t):
        row0 = pl.multiple_of(t * ts, ts)
        xf = x_buf[t].astype(f32)
        gl = jnp.sum(xf * gw_ref[...].astype(f32).reshape(1, d), axis=-1, keepdims=True)
        g_s[pl.ds(row0, ts), :] = jax.nn.sigmoid(gl)
        m = jnp.mean(xf, axis=-1, keepdims=True)
        xc = xf - m
        var = jnp.mean(xc * xc, axis=-1, keepdims=True)
        h = xc / jnp.sqrt(var + 1e-5)
        ht_s[:, pl.ds(row0, ts)] = h.T.astype(bf16)

    def attn_stats(t, first=False):
        row0 = pl.multiple_of(t * ts, ts)
        phi = lambda a: jnp.where(a > 0, a + 1.0, jnp.exp(a)) + 1e-6
        if first:
            def proj(j, then_start):
                wqkv_cp(j).wait()
                for cp in then_start:
                    cp.start()
                return jnp.dot(x_buf[t], wqkv_buf[:, pl.ds(j * d, d)],
                               preferred_element_type=f32)
            k = proj(1, (wqkv_cp(0), x_cp(1)))
            v = proj(2, (x_cp(2), w1_cp(0)))
            x_cp(1).wait()
            q = proj(0, ())
            norm_gate(1)
        else:
            qkv = jnp.dot(x_buf[t], wqkv_buf[...], preferred_element_type=f32)
            q = qkv[:, 0 * d:1 * d]
            k = qkv[:, 1 * d:2 * d]
            v = qkv[:, 2 * d:3 * d]
        pq_s[pl.ds(row0, ts), :] = phi(q).astype(bf16)
        pk = phi(k)
        z_s[...] += jnp.sum(pk, axis=0, keepdims=True)
        pkb = pk.astype(bf16)
        vb = v.astype(bf16)
        for gidx in range(ng):
            sl = slice(gidx * _LANES, (gidx + 1) * _LANES)
            kv_s[gidx] += jax.lax.dot_general(
                pkb[:, sl], vb[:, sl], (((0,), (0,)), ((), ())),
                preferred_element_type=f32)

    x_cp(0).wait()
    wqkv_cp(2).start()
    norm_gate(0)
    attn_stats(0, first=True)
    wo_cp.start()

    def phase_a(t, carry):
        @pl.when(t + 2 < nt)
        def _():
            x_cp(t + 2).start()

        @pl.when(t < nf)
        def _():
            w1_cp(t).start()

        @pl.when(t + 1 < nt)
        def _():
            x_cp(t + 1).wait()
            attn_stats(t)
            norm_gate(t + 1)

        @pl.when(t + 1 == nt)
        def _():
            wo_cp.wait()
            attn_stats(t)
            for gidx in range(ng):
                kvb = jnp.where(same, kv_s[gidx], 0.0).astype(bf16)
                m_s[pl.ds(gidx * _LANES, _LANES), :] = jnp.dot(
                    kvb, wo_buf[pl.ds(gidx * _LANES, _LANES), :],
                    preferred_element_type=f32).astype(bf16)
        return carry

    jax.lax.fori_loop(1, nt, phase_a, 0)

    for c in range(nt, nf):
        w1_cp(c).start()

    for c in range(nf):
        w1_cp(c).wait()
    for t in range(nt):
        w2_cp(t).start()

    def phase_b(c, carry):
        col0 = pl.multiple_of(c * cf, cf)
        u = jnp.dot(ht_s[...], w1_buf[c], preferred_element_type=f32)
        u = u + b1_ref[pl.ds(col0, cf)].astype(f32).reshape(1, cf)
        gu_s[:, pl.ds(col0, cf)] = jax.nn.gelu(u, approximate=True).astype(bf16)
        return carry

    jax.lax.fori_loop(0, nf, phase_b, 0, unroll=nf)

    ones_blk = jnp.where(same, 1.0, 0.0).astype(bf16)

    def phase_c(t, carry):
        w2_cp(t).wait()

        @pl.when(t >= 2)
        def _():
            out_cp(t - 2).wait()

        row0 = pl.multiple_of(t * ts, ts)
        w2t = w2_buf.at[t]
        parts = []
        yts = []
        for gidx in range(ng):
            sl = slice(gidx * _LANES, (gidx + 1) * _LANES)
            yts.append(jnp.dot(gu_s[sl, :], w2t[...], preferred_element_type=f32))
            pq = pq_s[pl.ds(row0, ts), sl].astype(f32)
            pqz = (pq * z_s[:, sl]).astype(bf16)
            den = jnp.dot(pqz, ones_blk, preferred_element_type=f32)
            parts.append((pq / (den + 1e-6)).astype(bf16))
        yt = jnp.concatenate(yts, axis=0) + b2_ref[pl.ds(row0, ts)].astype(f32).reshape(1, ts)
        b = yt.T
        pqn = jnp.concatenate(parts, axis=-1)
        a = jnp.dot(pqn, m_s[...], preferred_element_type=f32)
        g = g_s[pl.ds(row0, ts), :]
        out_buf[t % 2] = (g * a + (1.0 - g) * b).astype(out_buf.dtype)
        out_cp(t).start()
        return carry

    jax.lax.fori_loop(0, nt, phase_c, 0)
    out_cp(nt - 2).wait()
    out_cp(nt - 1).wait()


@jax.jit
def pallas_gated_mix__linear_attn_block__mixer_token_mlp__prompt_kernel(
    A_x: jax.Array,
    A_wqkv: jax.Array,
    A_wo: jax.Array,
    B_x: jax.Array,
    B_w1: jax.Array,
    B_b1: jax.Array,
    B_w2: jax.Array,
    B_b2: jax.Array,
    gate_w: jax.Array,
):
    del B_x
    bsz, s, d = A_x.shape
    assert bsz == 1
    f = B_w1.shape[1]
    n_heads = 32
    dh = d // n_heads
    ts = 256
    cf = 256
    nt = s // ts
    nf = f // cf
    ng = d // _LANES
    bf16 = jnp.bfloat16
    assert s % ts == 0 and f % cf == 0 and d % _LANES == 0 and _LANES % dh == 0
    assert nt >= 3

    x = A_x.reshape(s, d)
    b1, b2, gw = B_b1, B_b2, gate_w

    kern = functools.partial(_kernel, s=s, ts=ts, cf=cf, d=d, f=f, dh=dh)
    hbm = pl.BlockSpec(memory_space=pl.ANY)
    out = pl.pallas_call(
        kern,
        in_specs=[hbm, hbm, hbm, hbm, hbm,
                  pl.BlockSpec((f,), lambda: (0,)),
                  pl.BlockSpec((s,), lambda: (0,)),
                  pl.BlockSpec((d,), lambda: (0,))],
        out_specs=hbm,
        out_shape=jax.ShapeDtypeStruct((s, d), A_x.dtype),
        scratch_shapes=[
            pltpu.VMEM((nt, ts, d), bf16),
            pltpu.VMEM((d, 3 * d), bf16),
            pltpu.VMEM((d, d), bf16),
            pltpu.VMEM((nf, s, cf), bf16),
            pltpu.VMEM((nt, f, ts), bf16),
            pltpu.VMEM((d, s), bf16),
            pltpu.VMEM((s, d), bf16),
            pltpu.VMEM((s, 1), jnp.float32),
            pltpu.VMEM((ng, _LANES, _LANES), jnp.float32),
            pltpu.VMEM((1, d), jnp.float32),
            pltpu.VMEM((d, f), bf16),
            pltpu.VMEM((d, d), bf16),
            pltpu.VMEM((2, ts, d), A_x.dtype),
            pltpu.SemaphoreType.DMA((nt,)),
            pltpu.SemaphoreType.DMA((3,)),
            pltpu.SemaphoreType.DMA((1,)),
            pltpu.SemaphoreType.DMA((nf,)),
            pltpu.SemaphoreType.DMA((nt,)),
            pltpu.SemaphoreType.DMA((2,)),
        ],
        compiler_params=pltpu.CompilerParams(
            vmem_limit_bytes=100 * 1024 * 1024,
        ),
    )(x, A_wqkv, A_wo, B_w1, B_w2, b1, b2, gw)
    return out.reshape(1, s, d)
```
